```python
import jax
import jax.numpy as jnp

def _softmax(x, axis=-1):
    return jax.nn.softmax(x, axis=axis)
def _gelu(x):
    return jax.nn.gelu(x, approximate=True)
def _silu(x):
    return jax.nn.silu(x)
def _sigmoid(x):
    return jax.nn.sigmoid(x)
def _layernorm(x, axis=-1, eps=1e-5):
    m = jnp.mean(x, axis=axis, keepdims=True)
    v = jnp.var(x, axis=axis, keepdims=True)
    return (x - m) / jnp.sqrt(v + eps)
def _scatter_add(tgt, idx, src, axis=0):
    return tgt.at[idx].add(src)
def _segment_sum(src, seg, n):
    return jax.ops.segment_sum(src, seg, n)
class _Rng:
    def __init__(self, key):
        self._k = key
    def _next(self):
        self._k, sub = jax.random.split(self._k)
        return sub
    def normal(self, shape):
        return jax.random.normal(self._next(), shape, dtype=jnp.bfloat16)
    def randint(self, lo, hi, shape):
        return jax.random.randint(self._next(), shape, lo, hi, dtype=jnp.int32)
    def uniform(self, shape, lo=0.0, hi=1.0):
        return jax.random.uniform(self._next(), shape, jnp.bfloat16, lo, hi)
    def permutation(self, n):
        return jax.random.permutation(self._next(), n)


kernel_name = 'interleave_layers__sliding_block__sliding_local_dilated__prompt'

def setup_inputs():
    _rng = _Rng(jax.random.key(int.from_bytes(__import__("os").urandom(4), "little")))
    _w = (lambda a: (lambda t: t.astype(jnp.bfloat16) if jnp.issubdtype(t.dtype, jnp.floating) else t)(jnp.asarray(a)))
    def _A_setup():
        B, S, D = 1, 2048, 1024
        return {
            "x": _w((lambda *s: _rng.normal(s) * 0.05)(B, S, D)),
            "wqkv": _w((lambda *s: _rng.normal(s) * 0.05)(D, 3 * D)),
            "wo": _w((lambda *s: _rng.normal(s) * 0.05)(D, D)),
        }
    _A_in = _A_setup()

    def _B_setup():
        B, S, D = 1, 2048, 1024
        return {
            "x": _w((lambda *s: _rng.normal(s) * 0.05)(B, S, D)),
            "wqkv": _w((lambda *s: _rng.normal(s) * 0.05)(D, 3 * D)),
            "wo": _w((lambda *s: _rng.normal(s) * 0.05)(D, D)),
        }
    _B_in = _B_setup()

    return {
        "A_x": _A_in["x"],
        "A_wqkv": _A_in["wqkv"],
        "A_wo": _A_in["wo"],
        "B_x": _B_in["x"],
        "B_wqkv": _B_in["wqkv"],
        "B_wo": _B_in["wo"],
    }

def reference(A_x, A_wqkv, A_wo, B_x, B_wqkv, B_wo):
    def _A_ref(x, wqkv, wo):
        B, S, D = x.shape
        H = 32; Dh = D // H; W = 256
        qkv = (lambda x, *d: x.transpose(*d))((x @ wqkv).reshape(B, S, 3, H, Dh), 2, 0, 3, 1, 4)
        q, k, v = qkv[0], qkv[1], qkv[2]
        scores = jnp.einsum("bhqd,bhkd->bhqk", q, k) * (Dh ** -0.5)
        idx = jnp.arange(S)
        mask = (idx[:, None] - idx[None, :] >= 0) & (idx[:, None] - idx[None, :] < W)
        scores = jnp.where(mask[None, None], scores, -1e9)
        p = _softmax(scores, axis=-1)
        o = jnp.einsum("bhqk,bhkd->bhqd", p, v)
        return (lambda x, *d: x.transpose(*d))(o, 0, 2, 1, 3).reshape(B, S, D) @ wo

    def _B_ref(x, wqkv, wo):
        B, S, D = x.shape
        H = 32; Dh = D // H
        W, dil = 8, 2
        qkv = (lambda x, *d: x.transpose(*d))((x @ wqkv).reshape(B, S, 3, H, Dh), 2, 0, 3, 1, 4)
        q, k, v = qkv[0], qkv[1], qkv[2]
        scale = Dh ** -0.5
        pos = jnp.arange(S)
        off = jnp.arange(W) * dil
        idx = pos[:, None] - off[None, :]
        mask = idx >= 0
        idx_c = jnp.where(mask, idx, 0).reshape(-1)
        kg = k[:, :, idx_c, :].reshape(B, H, S, W, Dh)
        vg = v[:, :, idx_c, :].reshape(B, H, S, W, Dh)
        logits = jnp.einsum("bhsd,bhswd->bhsw", q, kg) * scale
        logits = jnp.where(mask[None, None, :, :], logits, -1e9)
        attn = _softmax(logits, axis=-1)
        o = jnp.einsum("bhsw,bhswd->bhsd", attn, vg)
        return (lambda x, *d: x.transpose(*d))(o, 0, 2, 1, 3).reshape(B, S, D) @ wo

    x = A_x
    x = x + _A_ref(_layernorm(x, axis=-1), A_wqkv, A_wo)
    x = x + _B_ref(_layernorm(x, axis=-1), B_wqkv, B_wo)
    x = x + _A_ref(_layernorm(x, axis=-1), A_wqkv, A_wo)
    x = x + _B_ref(_layernorm(x, axis=-1), B_wqkv, B_wo)
    return x
```

```python
import functools
import math

import jax
import jax.numpy as jnp
import numpy as np
import jax.experimental.pallas as pl
import jax.experimental.pallas.tpu as pltpu

S = 2048
D = 1024
G = 8
DH = 32
WIN_A = 256
EPS = 1e-5
QSCALE = float(DH ** -0.5 * math.log2(math.e))
NT = (((1,), (1,)), ((), ()))
TM = 256
NB = 3

f32 = jnp.float32
bf16 = jnp.bfloat16


def _head_masked(q4):
    qi = pltpu.bitcast(q4, jnp.int32)
    lane = jax.lax.broadcasted_iota(jnp.int32, qi.shape, 1)
    return jnp.concatenate(
        [pltpu.bitcast(qi & jnp.where((lane // DH) == h, -1, 0), bf16) for h in range(4)], axis=0)


def _after(tok, m):
    return jnp.where(tok > jnp.inf, 0.0, m)


def _layernorm(x):
    m = jnp.mean(x, axis=-1, keepdims=True)
    xc = x - m
    v = jnp.mean(xc * xc, axis=-1, keepdims=True)
    return xc * jax.lax.rsqrt(v + EPS)


def _attn_a(g, q_s, k_s, vt_s, o_s, sbufs, pbufs, lbufs):
    row = jax.lax.broadcasted_iota(jnp.int32, (128, 128), 0)
    lane = jax.lax.broadcasted_iota(jnp.int32, (128, 128), 1)
    upper = row > lane
    nj = S // 128
    NC, CH = 4, 96
    tok = {}

    def qk_chunk(j, c, qbd):
        lo = max(0, 2 - j) * 128
        r0, r1 = max(c * CH, lo), (c + 1) * CH
        if r0 >= r1:
            return
        kw = k_s[g, j * 128 - 256 + r0: j * 128 - 256 + r1, :]
        st = jax.lax.dot_general(kw, qbd, NT, preferred_element_type=f32)
        sbufs[j % NB][r0:r1, :] = st
        tok[c] = st[0:1, 0:128]

    def softmax(j, h):
        sb, pb, lb = sbufs[j % NB], pbufs[j % NB], lbufs[j % NB]
        cs = slice(h * 128, (h + 1) * 128)
        dep = (lambda m: _after(tok[h], m)) if h in tok else (lambda m: m)
        if j >= 1:
            s1 = sb[128:256, cs]
            if j >= 2:
                s0 = jnp.where(upper, sb[0:128, cs], sb[256:384, cs])
            else:
                s0 = jnp.where(upper, -jnp.inf, sb[256:384, cs])
            m = dep(jnp.maximum(jnp.max(s0, axis=0, keepdims=True), jnp.max(s1, axis=0, keepdims=True)))
            p0 = jnp.exp2(s0 - m)
            p1 = jnp.exp2(s1 - m)
            l = jnp.sum(p0, axis=0, keepdims=True) + jnp.sum(p1, axis=0, keepdims=True)
            if j >= 2:
                pb[h, 0:128, :] = jnp.where(upper, p0, 0.0).astype(bf16)
                pb[h, 256:384, :] = jnp.where(upper, 0.0, p0).astype(bf16)
            else:
                pb[h, 256:384, :] = p0.astype(bf16)
            pb[h, 128:256, :] = p1.astype(bf16)
        else:
            s0 = jnp.where(upper, -jnp.inf, sb[256:384, cs])
            m = dep(jnp.max(s0, axis=0, keepdims=True))
            p0 = jnp.exp2(s0 - m)
            l = jnp.sum(p0, axis=0, keepdims=True)
            pb[h, 256:384, :] = p0.astype(bf16)
        lb[:, cs] = jnp.broadcast_to(1.0 / l, (8, 128))

    def pv(j):
        pb, lb = pbufs[j % NB], lbufs[j % NB]
        lo = max(0, 2 - j) * 128
        outs = []
        for h in range(4):
            vth = vt_s[g, h * DH:(h + 1) * DH, j * 128 - 256 + lo: j * 128 + 128]
            ot = jnp.dot(vth, pb[h, lo:384, :], preferred_element_type=f32)
            outs.append(ot * lb[0:1, h * 128:(h + 1) * 128])
        o_s[g, j * 128:(j + 1) * 128, :] = jnp.concatenate(outs, axis=0).T.astype(bf16)

    for n in range(nj + 2):
        tok.clear()
        if n < nj:
            qbd = _head_masked(q_s[g, n * 128:(n + 1) * 128, :])
            for c in range(NC):
                qk_chunk(n, c, qbd)
        if 0 <= n - 1 < nj:
            for h in range(4):
                softmax(n - 1, h)
        if 0 <= n - 2 < nj:
            pv(n - 2)


def _attn_b(g, q_s, k_s, vt_s, o_s):
    row = jax.lax.broadcasted_iota(jnp.int32, (144, 128), 0)
    lane = jax.lax.broadcasted_iota(jnp.int32, (144, 128), 1)
    dist = lane + 16 - row
    bias = jnp.where((dist >= 0) & (dist <= 14) & ((dist & 1) == 0), 0.0, -jnp.inf).astype(f32)
    for j in range(S // 128):
        qbd = _head_masked(q_s[g, j * 128:(j + 1) * 128, :])
        lo = 16 if j == 0 else 0
        kw = k_s[g, j * 128 - 16 + lo: j * 128 + 128, :]
        st = jax.lax.dot_general(kw, qbd, NT, preferred_element_type=f32)
        outs = []
        for h in range(4):
            s = st[:, h * 128:(h + 1) * 128] + bias[lo:, :]
            m = jnp.max(s, axis=0, keepdims=True)
            p = jnp.exp2(s - m)
            l = jnp.sum(p, axis=0, keepdims=True)
            pb = p.astype(bf16)
            ot = jnp.dot(vt_s[g, h * DH:(h + 1) * DH, j * 128:(j + 1) * 128], pb[16 - lo:, :],
                         preferred_element_type=f32)
            if j > 0:
                pz = jnp.concatenate([jnp.zeros((112, 128), bf16), pb[0:16, :]], axis=0)
                ot = ot + jnp.dot(vt_s[g, h * DH:(h + 1) * DH, j * 128 - 128:j * 128], pz,
                                  preferred_element_type=f32)
            outs.append(ot * (1.0 / l))
        o_s[g, j * 128:(j + 1) * 128, :] = jnp.concatenate(outs, axis=0).T.astype(bf16)


def _kernel(x_hbm, awqkv_hbm, awo_hbm, bwqkv_hbm, bwo_hbm, out_hbm,
            xin, xres, wqk, wvt, wv_raw, wo, q_s, k_s, vt_s, o_s, sems, *bufs):
    sbufs, pbufs, lbufs = bufs[0:NB], bufs[NB:2 * NB], bufs[2 * NB:3 * NB]

    def cp(src, dst, i):
        return pltpu.make_async_copy(src, dst, sems.at[i])

    copies = [
        cp(x_hbm, xin, 0),
        cp(awqkv_hbm.at[:, 0:2 * D], wqk.at[0], 1),
        cp(awqkv_hbm.at[:, 2 * D:3 * D], wv_raw.at[0], 2),
        cp(awo_hbm, wo.at[0], 3),
        cp(bwqkv_hbm.at[:, 0:2 * D], wqk.at[1], 4),
        cp(bwqkv_hbm.at[:, 2 * D:3 * D], wv_raw.at[1], 5),
        cp(bwo_hbm, wo.at[1], 6),
    ]
    for c in copies:
        c.start()
    copies[0].wait()

    @pl.loop(0, S // TM)
    def _(i):
        r = pl.ds(pl.multiple_of(i * TM, TM), TM)
        xres[r, :] = xin[r, :].astype(f32)

    for c in copies[1:]:
        c.wait()
    for w in range(2):
        for a in range(G):
            for b in range(G):
                wvt[w, a * 128:(a + 1) * 128, b * 128:(b + 1) * 128] = (
                    wv_raw[w, b * 128:(b + 1) * 128, a * 128:(a + 1) * 128].astype(f32).T.astype(bf16))

    def in_proj(w):
        @pl.loop(0, S // TM)
        def _(i):
            r0 = pl.multiple_of(i * TM, TM)
            r = pl.ds(r0, TM)
            xn = _layernorm(xres[r, :]).astype(bf16)
            qk = jnp.dot(xn, wqk[w], preferred_element_type=f32)
            for g in range(G):
                q_s[g, r, :] = (qk[:, g * 128:(g + 1) * 128] * QSCALE).astype(bf16)
                k_s[g, r, :] = qk[:, D + g * 128:D + (g + 1) * 128].astype(bf16)
            vt = jax.lax.dot_general(wvt[w], xn, NT, preferred_element_type=f32)
            for g in range(G):
                vt_s[g, :, r] = vt[g * 128:(g + 1) * 128, :].astype(bf16)

    def out_proj(w):
        @pl.loop(0, S // TM)
        def _(i):
            r = pl.ds(pl.multiple_of(i * TM, TM), TM)
            o = jnp.concatenate([o_s[g, r, :] for g in range(G)], axis=1)
            xres[r, :] = xres[r, :] + jnp.dot(o, wo[w], preferred_element_type=f32)

    @pl.loop(0, 2)
    def _(rep):
        in_proj(0)

        @pl.loop(0, G)
        def _(g):
            _attn_a(g, q_s, k_s, vt_s, o_s, sbufs, pbufs, lbufs)

        out_proj(0)
        in_proj(1)

        @pl.loop(0, G)
        def _(g):
            _attn_b(g, q_s, k_s, vt_s, o_s)

        out_proj(1)

    @pl.loop(0, S // TM)
    def _(i):
        r = pl.ds(pl.multiple_of(i * TM, TM), TM)
        xin[r, :] = xres[r, :].astype(bf16)

    c = cp(xin, out_hbm, 0)
    c.start()
    c.wait()


@jax.jit
def pallas_interleave_layers__sliding_block__sliding_local_dilated__prompt_kernel(
    A_x: jax.Array,
    A_wqkv: jax.Array,
    A_wo: jax.Array,
    B_x: jax.Array,
    B_wqkv: jax.Array,
    B_wo: jax.Array,
):
    del B_x
    any_spec = pl.BlockSpec(memory_space=pl.ANY)
    out = pl.pallas_call(
        _kernel,
        out_shape=jax.ShapeDtypeStruct((S, D), bf16),
        in_specs=[any_spec] * 5,
        out_specs=any_spec,
        scratch_shapes=[
            pltpu.VMEM((S, D), bf16),
            pltpu.VMEM((S, D), f32),
            pltpu.VMEM((2, D, 2 * D), bf16),
            pltpu.VMEM((2, D, D), bf16),
            pltpu.VMEM((2, D, D), bf16),
            pltpu.VMEM((2, D, D), bf16),
            pltpu.VMEM((G, S, 128), bf16),
            pltpu.VMEM((G, S, 128), bf16),
            pltpu.VMEM((G, 128, S), bf16),
            pltpu.VMEM((G, S, 128), bf16),
            pltpu.SemaphoreType.DMA((8,)),
        ] + [pltpu.VMEM((384, 512), f32)] * NB
          + [pltpu.VMEM((4, 384, 128), bf16)] * NB
          + [pltpu.VMEM((8, 512), f32)] * NB,
        compiler_params=pltpu.CompilerParams(vmem_limit_bytes=120 * 1024 * 1024),
    )(A_x.reshape(S, D), A_wqkv, A_wo, B_wqkv, B_wo)
    return out.reshape(1, S, D)
```

```python
import functools
import math

import jax
import jax.numpy as jnp
import numpy as np
import jax.experimental.pallas as pl
import jax.experimental.pallas.tpu as pltpu

S = 2048
D = 1024
G = 8
DH = 32
WIN_A = 256
EPS = 1e-5
QSCALE = float(DH ** -0.5 * math.log2(math.e))
NT = (((1,), (1,)), ((), ()))
LN_ROWS = 64
TM = 512
NB = 4

f32 = jnp.float32
bf16 = jnp.bfloat16


def _head_masked(q4):
    qi = pltpu.bitcast(q4, jnp.int32)
    lane = jax.lax.broadcasted_iota(jnp.int32, qi.shape, 1)
    return jnp.concatenate(
        [pltpu.bitcast(qi & jnp.where((lane // DH) == h, -1, 0), bf16) for h in range(4)], axis=0)


def _after(tok, m):
    return jnp.where(tok > jnp.inf, 0.0, m)


def _layernorm(x):
    m = jnp.mean(x, axis=-1, keepdims=True)
    xc = x - m
    v = jnp.mean(xc * xc, axis=-1, keepdims=True)
    return xc * jax.lax.rsqrt(v + EPS)


def _attn_a(g, q_s, k_s, vt_s, o_s, sbufs, pbufs, lbufs):
    row = jax.lax.broadcasted_iota(jnp.int32, (128, 128), 0)
    lane = jax.lax.broadcasted_iota(jnp.int32, (128, 128), 1)
    upper = row > lane
    nj = S // 128
    NC = 4; CH = 384 // NC; MG = 2; TR = 0; L2 = 2; TS = -1
    tok = {}

    def qk_chunk(j, c, qbd):
        if j >= 2 and MG and c < MG:
            w = 128 // MG
            b = j * 128 - 256 + c * w
            kw = jnp.concatenate([k_s[g, b:b + w, :], k_s[g, b + 256:b + 256 + w, :]], axis=0)
            st = jax.lax.dot_general(kw, qbd, NT, preferred_element_type=f32)
            up = jnp.concatenate([upper[c * w:(c + 1) * w]] * 4, axis=1)
            sbufs[j % NB][c * w:(c + 1) * w, :] = jnp.where(up, st[0:w], st[w:2 * w])
            tok[c] = st[TR:TR + 1, 0:128]
            return
        if j >= 2 and MG:
            n1 = NC - MG
            w = 128 // n1
            r0 = 128 + (c - MG) * w
            kw = k_s[g, j * 128 - 256 + r0: j * 128 - 256 + r0 + w, :]
            st = jax.lax.dot_general(kw, qbd, NT, preferred_element_type=f32)
            sbufs[j % NB][r0:r0 + w, :] = st
            tr = min(TR, w - 1); tok[c] = st[tr:tr + 1, 0:128]
            return
        lo = max(0, 2 - j) * 128
        r0, r1 = max(c * CH, lo), (c + 1) * CH
        if r0 >= r1:
            return
        kw = k_s[g, j * 128 - 256 + r0: j * 128 - 256 + r1, :]
        st = jax.lax.dot_general(kw, qbd, NT, preferred_element_type=f32)
        sbufs[j % NB][r0:r1, :] = st
        tr = min(TR, r1 - r0 - 1); tok[c] = st[tr:tr + 1, 0:128]

    def softmax(j, h):
        sb, pb, lb = sbufs[j % NB], pbufs[j % NB], lbufs[j % NB]
        cs = slice(h * 128, (h + 1) * 128)
        th = h * NC // 4 + TS
        dep = (lambda m: _after(tok[th], m)) if th in tok else (lambda m: m)
        if j >= 1:
            s1 = sb[128:256, cs]
            if j >= 2:
                s0 = sb[0:128, cs] if MG else jnp.where(upper, sb[0:128, cs], sb[256:384, cs])
            else:
                s0 = jnp.where(upper, -jnp.inf, sb[256:384, cs])
            m = dep(jnp.maximum(jnp.max(s0, axis=0, keepdims=True), jnp.max(s1, axis=0, keepdims=True)))
            p0 = jnp.exp2(s0 - m)
            p1 = jnp.exp2(s1 - m)
            l = jnp.sum(p0, axis=0, keepdims=True) + jnp.sum(p1, axis=0, keepdims=True)
            if j >= 2:
                pb[h, 0:128, :] = jnp.where(upper, p0, 0.0).astype(bf16)
                pb[h, 256:384, :] = jnp.where(upper, 0.0, p0).astype(bf16)
            else:
                pb[h, 256:384, :] = p0.astype(bf16)
            pb[h, 128:256, :] = p1.astype(bf16)
        else:
            s0 = jnp.where(upper, -jnp.inf, sb[256:384, cs])
            m = dep(jnp.max(s0, axis=0, keepdims=True))
            p0 = jnp.exp2(s0 - m)
            l = jnp.sum(p0, axis=0, keepdims=True)
            pb[h, 256:384, :] = p0.astype(bf16)
        lb[:, cs] = jnp.broadcast_to(1.0 / l, (8, 128))

    def pv(j):
        pb, lb = pbufs[j % NB], lbufs[j % NB]
        lo = max(0, 2 - j) * 128
        outs = []
        for h in range(4):
            vth = vt_s[g, h * DH:(h + 1) * DH, j * 128 - 256 + lo: j * 128 + 128]
            ot = jnp.dot(vth, pb[h, lo:384, :], preferred_element_type=f32)
            outs.append(ot * lb[0:1, h * 128:(h + 1) * 128])
        o_s[g, j * 128:(j + 1) * 128, :] = jnp.concatenate(outs, axis=0).T.astype(bf16)

    for n in range(nj + L2):
        tok.clear()
        if n < nj:
            qbd = _head_masked(q_s[g, n * 128:(n + 1) * 128, :])
            for c in range(NC):
                qk_chunk(n, c, qbd)
        if 0 <= n - 1 < nj:
            for h in range(4):
                softmax(n - 1, h)
        if 0 <= n - L2 < nj:
            pv(n - L2)


def _attn_b(g, q_s, k_s, v_s, o_s):
    row = jax.lax.broadcasted_iota(jnp.int32, (128, 128), 0) & 31
    lane = jax.lax.broadcasted_iota(jnp.int32, (128, 128), 1) & 31
    dist = (lane - row) & 31
    ok = (dist <= 14) & ((dist & 1) == 0)
    bias = jnp.where(ok, 0.0, -jnp.inf).astype(f32)
    lane_full = jax.lax.broadcasted_iota(jnp.int32, (128, 128), 1)
    bias0 = jnp.where(ok & ((lane_full >= 32) | (row <= lane)), 0.0, -jnp.inf).astype(f32)
    qi = jax.lax.broadcasted_iota(jnp.int32, (16, 128), 0)
    kc = jax.lax.broadcasted_iota(jnp.int32, (16, 128), 1) & 31
    prev_tile = kc > qi
    nt, nj = S // 32, S // 128
    st, pr, out = {}, {}, {}

    def qk(t):
        rows = 48 if t < nt - 1 else 32
        kbd = _head_masked(k_s[g, t * 32:(t + 1) * 32, :])
        st[t] = jax.lax.dot_general(q_s[g, t * 32:t * 32 + rows, :], kbd, NT, preferred_element_type=f32)

    def softmax(j):
        parts = []
        for t in range(4 * j, 4 * j + 4):
            top = st[t][0:16]
            if t > 0:
                top = jnp.where(prev_tile, st[t - 1][32:48], top)
            parts += [top, st[t][16:32]]
        s = jnp.concatenate(parts, axis=0).T + (bias0 if j == 0 else bias)
        pn = []
        for h in range(4):
            sh = s[h * 32:(h + 1) * 32]
            p = jnp.exp2(sh - jnp.max(sh, axis=0, keepdims=True))
            pn.append(p * (1.0 / jnp.sum(p, axis=0, keepdims=True)))
        pr[j] = jnp.concatenate(pn, axis=0).T

    def pv(t):
        u = t % 4
        pj = pr[t // 4]
        lhs = [jnp.where(prev_tile, 0.0, pj[u * 32:u * 32 + 16]), pj[u * 32 + 16:u * 32 + 32]]
        if t < nt - 1:
            pn = pr[(t + 1) // 4]
            un = (t + 1) % 4
            lhs.append(jnp.where(prev_tile, pn[un * 32:un * 32 + 16], 0.0))
        vbd = _head_masked(v_s[g, t * 32:(t + 1) * 32, :])
        out[t] = jnp.dot(jnp.concatenate(lhs, axis=0).astype(bf16), vbd, preferred_element_type=f32)
        top = out[t][0:16]
        if t > 0:
            top = top + out[t - 1][32:48]
        o_s[g, t * 32:(t + 1) * 32, :] = jnp.concatenate([top, out[t][16:32]], axis=0).astype(bf16)

    l1, l2 = 1, 8
    for n in range(nj + l2):
        if n < nj:
            for t in range(4 * n, 4 * n + 4):
                qk(t)
        if 0 <= n - l1 < nj:
            softmax(n - l1)
        if n >= l2:
            for t in range(max(0, 4 * (n - l2) - 1), 4 * (n - l2) + 3):
                pv(t)
    pv(nt - 1)


def _kernel(x_hbm, awqkv_hbm, awo_hbm, bwqkv_hbm, bwo_hbm, out_hbm,
            xin, xres, xn_s, wqk, wvt, wv_raw, wo, q_s, k_s, vt_s, v_s, o_s, sems, out_sem, *bufs):
    sbufs, pbufs, lbufs = bufs[0:NB], bufs[NB:2 * NB], bufs[2 * NB:3 * NB]
    nblk = S // TM

    def cp(src, dst, i):
        return pltpu.make_async_copy(src, dst, sems.at[i])

    first = [
        cp(x_hbm, xin, 0),
        cp(awqkv_hbm.at[:, 0:2 * D], wqk.at[0], 1),
        cp(awqkv_hbm.at[:, 2 * D:3 * D], wv_raw.at[0], 2),
    ]
    later = [
        cp(awo_hbm, wo.at[0], 3),
        cp(bwqkv_hbm.at[:, 0:2 * D], wqk.at[1], 4),
        cp(bwqkv_hbm.at[:, 2 * D:3 * D], wv_raw.at[1], 5),
        cp(bwo_hbm, wo.at[1], 6),
    ]
    first[0].start()
    first[2].start()
    first[0].wait()
    first[1].start()

    @pl.loop(0, nblk)
    def _(i):
        r = pl.ds(pl.multiple_of(i * TM, TM), TM)
        xres[r, :] = xin[r, :].astype(f32)

    def norm_block(i):
        toks = []
        for c in range(TM // LN_ROWS):
            r = pl.ds(pl.multiple_of(i * TM + c * LN_ROWS, LN_ROWS), LN_ROWS)
            y = _layernorm(xres[r, :])
            xn_s[r, :] = y.astype(bf16)
            toks.append(y[LN_ROWS - 1:LN_ROWS, D - 128:D])
        return toks

    first[2].wait()
    for a in range(G):
        for b in range(G):
            wvt[a * 128:(a + 1) * 128, b * 128:(b + 1) * 128] = (
                wv_raw[0, b * 128:(b + 1) * 128, a * 128:(a + 1) * 128].astype(f32).T.astype(bf16))
    first[1].wait()
    for c in later:
        c.start()

    def in_proj(w, prologue=True):
        if prologue:
            norm_block(0)

        @pl.loop(0, nblk)
        def _(i):
            r = pl.ds(pl.multiple_of(i * TM, TM), TM)
            xn = xn_s[r, :]
            qk = jnp.dot(xn, wqk[w], preferred_element_type=f32)
            toks = norm_block((i + 1) % nblk)
            for g in range(G):
                qscale = _after(toks[g * len(toks) // G], jnp.full((1, 128), QSCALE, f32))
                q_s[g, r, :] = (qk[:, g * 128:(g + 1) * 128] * qscale).astype(bf16)
                k_s[g, r, :] = qk[:, D + g * 128:D + (g + 1) * 128].astype(bf16)
            if w == 0:
                vt = jax.lax.dot_general(wvt[...], xn, NT, preferred_element_type=f32)
                for g in range(G):
                    vt_s[g, :, r] = vt[g * 128:(g + 1) * 128, :].astype(bf16)
            else:
                v = jnp.dot(xn, wv_raw[1], preferred_element_type=f32)
                for g in range(G):
                    v_s[g, r, :] = v[:, g * 128:(g + 1) * 128].astype(bf16)

    def out_copy(i):
        r = pl.ds(pl.multiple_of(i * TM, TM), TM)
        return pltpu.make_async_copy(xin.at[r, :], out_hbm.at[r, :], out_sem.at[0])

    def out_proj(w, rep):
        @pl.loop(0, nblk)
        def _(i):
            r = pl.ds(pl.multiple_of(i * TM, TM), TM)
            o = jnp.concatenate([o_s[g, r, :] for g in range(G)], axis=1)
            x = xres[r, :] + jnp.dot(o, wo[w], preferred_element_type=f32)
            xres[r, :] = x
            if w == 1:
                xin[r, :] = x.astype(bf16)

                @pl.when(rep == 1)
                def _():
                    out_copy(i).start()

    @pl.loop(0, 2)
    def _(rep):
        in_proj(0)

        @pl.loop(0, G)
        def _(g):
            _attn_a(g, q_s, k_s, vt_s, o_s, sbufs, pbufs, lbufs)

        @pl.when(rep == 0)
        def _():
            for c in later:
                c.wait()

        out_proj(0, rep)
        in_proj(1)

        @pl.loop(0, G)
        def _(g):
            _attn_b(g, q_s, k_s, v_s, o_s)

        out_proj(1, rep)

    for i in range(nblk):
        out_copy(i).wait()


@jax.jit
def pallas_interleave_layers__sliding_block__sliding_local_dilated__prompt_kernel(
    A_x: jax.Array,
    A_wqkv: jax.Array,
    A_wo: jax.Array,
    B_x: jax.Array,
    B_wqkv: jax.Array,
    B_wo: jax.Array,
):
    del B_x
    any_spec = pl.BlockSpec(memory_space=pl.ANY)
    out = pl.pallas_call(
        _kernel,
        out_shape=jax.ShapeDtypeStruct((S, D), bf16),
        in_specs=[any_spec] * 5,
        out_specs=any_spec,
        scratch_shapes=[
            pltpu.VMEM((S, D), bf16),
            pltpu.VMEM((S, D), f32),
            pltpu.VMEM((S, D), bf16),
            pltpu.VMEM((2, D, 2 * D), bf16),
            pltpu.VMEM((D, D), bf16),
            pltpu.VMEM((2, D, D), bf16),
            pltpu.VMEM((2, D, D), bf16),
            pltpu.VMEM((G, S, 128), bf16),
            pltpu.VMEM((G, S, 128), bf16),
            pltpu.VMEM((G, 128, S), bf16),
            pltpu.VMEM((G, S, 128), bf16),
            pltpu.VMEM((G, S, 128), bf16),
            pltpu.SemaphoreType.DMA((8,)),
            pltpu.SemaphoreType.DMA((1,)),
        ] + [pltpu.VMEM((384, 512), f32)] * NB
          + [pltpu.VMEM((4, 384, 128), bf16)] * NB
          + [pltpu.VMEM((8, 512), f32)] * NB,
        compiler_params=pltpu.CompilerParams(vmem_limit_bytes=120 * 1024 * 1024),
    )(A_x.reshape(S, D), A_wqkv, A_wo, B_wqkv, B_wo)
    return out.reshape(1, S, D)
```
